```python
import os as _os
_os.environ.setdefault("JAX_PLATFORMS", "cpu")
import jax
import jax.numpy as jnp

def _softmax(x, axis=-1):
    return jax.nn.softmax(x, axis=axis)
def _gelu(x):
    return jax.nn.gelu(x, approximate=True)
def _silu(x):
    return jax.nn.silu(x)
def _sigmoid(x):
    return jax.nn.sigmoid(x)
def _layernorm(x, axis=-1, eps=1e-5):
    m = jnp.mean(x, axis=axis, keepdims=True)
    v = jnp.var(x, axis=axis, keepdims=True)
    return (x - m) / jnp.sqrt(v + eps)
def _scatter_add(tgt, idx, src, axis=0):
    return tgt.at[idx].add(src)
def _segment_sum(src, seg, n):
    return jax.ops.segment_sum(src, seg, n)
class _Rng:
    def __init__(self, key):
        self._k = key
    def _next(self):
        self._k, sub = jax.random.split(self._k)
        return sub
    def normal(self, shape):
        return jax.random.normal(self._next(), shape, dtype=jnp.bfloat16)
    def randint(self, lo, hi, shape):
        return jax.random.randint(self._next(), shape, lo, hi, dtype=jnp.int32)
    def uniform(self, shape, lo=0.0, hi=1.0):
        return jax.random.uniform(self._next(), shape, jnp.bfloat16, lo, hi)
    def permutation(self, n):
        return jax.random.permutation(self._next(), n)


kernel_name = 'gated_mix__mha_block__linear_kernel_hedgehog__prompt'

def setup_inputs():
    _rng = _Rng(jax.random.key(int.from_bytes(__import__("os").urandom(4), "little")))
    _w = (lambda a: (lambda t: t.astype(jnp.bfloat16) if jnp.issubdtype(t.dtype, jnp.floating) else t)(jnp.asarray(a)))
    def _A_setup():
        B, S, D, H = 1, 2048, 640, 32
        return {
            "x": _w((lambda *s: _rng.normal(s) * 0.05)(B, S, D)),
            "wqkv": _w((lambda *s: _rng.normal(s) * 0.4)(D, 3 * D)),
            "wo": _w((lambda *s: _rng.normal(s) * 0.05)(D, D)),
        }
    _A_in = _A_setup()

    def _B_setup():
        B, S, D, H = 1, 2048, 640, 32
        Dh = D // H
        return {
            "x": _w((lambda *s: _rng.normal(s) * 0.05)(B, S, D)),
            "wqkv": _w((lambda *s: _rng.normal(s) * 0.8)(D, 3 * D)),
            "w_phi": _w((lambda *s: _rng.normal(s) * 0.8)(H, Dh, Dh) * (Dh ** -0.5)),
            "wo": _w((lambda *s: _rng.normal(s) * 0.05)(D, D)),
        }
    _B_in = _B_setup()

    return {
        "A_x": _A_in["x"],
        "A_wqkv": _A_in["wqkv"],
        "A_wo": _A_in["wo"],
        "B_x": _B_in["x"],
        "B_wqkv": _B_in["wqkv"],
        "B_w_phi": _B_in["w_phi"],
        "B_wo": _B_in["wo"],
        "gate_w": _w((lambda *s: _rng.normal(s) * 0.05)(640) * 16.0),
    }

def reference(A_x, A_wqkv, A_wo, B_x, B_wqkv, B_w_phi, B_wo, gate_w):
    def _A_ref(x, wqkv, wo):
        B, S, D = x.shape
        H = 32
        Dh = D // H
        qkv = (lambda x, *d: x.transpose(*d))((x @ wqkv).reshape(B, S, 3, H, Dh), 2, 0, 3, 1, 4)
        q, k, v = qkv[0], qkv[1], qkv[2]
        scores = jnp.einsum("bhqd,bhkd->bhqk", q, k) * (Dh ** -0.5)
        p = _softmax(scores, axis=-1)
        o = jnp.einsum("bhqk,bhkd->bhqd", p, v)
        return (lambda x, *d: x.transpose(*d))(o, 0, 2, 1, 3).reshape(B, S, D) @ wo

    def _B_ref(x, wqkv, w_phi, wo):
        B, S, D = x.shape
        H = 32; Dh = D // H
        qkv = (lambda x, *d: x.transpose(*d))((x @ wqkv).reshape(B, S, 3, H, Dh), 2, 0, 3, 1, 4)
        q, k, v = qkv[0], qkv[1], qkv[2]
        pq = jnp.einsum("bhsd,hdf->bhsf", q, w_phi)
        pk = jnp.einsum("bhsd,hdf->bhsf", k, w_phi)
        phi_q = jnp.concatenate([_softmax(pq, axis=-1), _softmax(-pq, axis=-1)], axis=-1)
        phi_k = jnp.concatenate([_softmax(pk, axis=-1), _softmax(-pk, axis=-1)], axis=-1)
        kv = jnp.einsum("bhsf,bhsd->bhfd", phi_k, v)
        z  = jnp.einsum("bhsf->bhf", phi_k)
        num = jnp.einsum("bhqf,bhfd->bhqd", phi_q, kv)
        den = jnp.einsum("bhqf,bhf->bhq", phi_q, z)[..., None] + 1e-6
        o = num / den
        return (lambda x, *d: x.transpose(*d))(o, 0, 2, 1, 3).reshape(B, S, D) @ wo

    x = A_x
    g = _sigmoid((x * gate_w).sum(-1, keepdims=True))
    a = _A_ref(x, A_wqkv, A_wo)
    b = _B_ref(x, B_wqkv, B_w_phi, B_wo)
    return g * a + (1 - g) * b
```

```python
import functools

import jax
import jax.numpy as jnp
import jax.experimental.pallas as pl
import jax.experimental.pallas.tpu as pltpu

S = 2048
D = 640
H = 32
DH = 20
TQ = 512
NQ = S // TQ
CK = 128
NC = S // CK
SKEW = 3
MQ = 12
ST = 17
TO = 512
OUT_TAIL = (384, 128)
LOG2E = 1.4426950408889634
QSCALE = (DH ** -0.5) * LOG2E

F32 = jnp.float32
BF16 = jnp.bfloat16
I32 = jnp.int32
U32 = jnp.uint32

NT = (((1,), (1,)), ((), ()))
TN = (((0,), (0,)), ((), ()))


def _dot(a, b, dims=None):
    if dims is None:
        return jnp.dot(a, b, preferred_element_type=F32)
    return jax.lax.dot_general(a, b, dims, preferred_element_type=F32)


def _round_bf16(x):
    return x.astype(BF16).astype(F32)


def _as_u32(x):
    return pltpu.bitcast(x, U32)


def _as_bf16(x):
    return pltpu.bitcast(x, BF16)


def _recip(x):
    r = pl.reciprocal(x, approx=True)
    return r * (2.0 - x * r)


def _pair_layout(vt):
    t = vt.shape[1]
    v3 = vt.reshape(H // 2, 2 * DH, t)
    mid = v3[:, 16:24, :]
    sub = jax.lax.broadcasted_iota(I32, mid.shape, 1)
    ev = jnp.where(sub < 4, mid, jnp.where(sub == 4, 1.0, 0.0))
    od = jnp.where(sub >= 4, mid, jnp.where(sub == 0, 1.0, 0.0))
    out = jnp.concatenate([v3[:, 0:16, :], ev, od, v3[:, 24:40, :]], axis=1)
    return out.reshape(H * 24, t)


def _kernel(xa_h, wa_h, woa_h, wb_h, wphi_h, wob_h, gate_h, out_h,
            xa_s, w_s, wo_s, wphi_s, gate_s,
            wT, wbT, f_s, acc_s,
            kw, qT, vtpA, vtpB, g_s, otA, otB,
            s2, mA, mB, zv, phq, phk, out_s, sems, osems):
    def cp(src, dst, i):
        return pltpu.make_async_copy(src, dst, sems.at[i])

    def xa_cp(c):
        return cp(xa_h.at[pl.ds(c * TQ, TQ)], xa_s.at[pl.ds(c * TQ, TQ)], c)

    wb_s = w_s.at[0]
    wa_s = w_s.at[1]

    def w_cp(src_h, slot, part, sem):
        return cp(src_h.at[:, pl.ds(D * part, D)], w_s.at[slot, :, pl.ds(D * part, D)], sem)

    wbq_cp = w_cp(wb_h, 0, 0, NQ)
    wbk_cp = w_cp(wb_h, 0, 1, NQ + 1)
    wak_cp = w_cp(wa_h, 1, 1, NQ + 6)
    late_cp = [w_cp(wa_h, 1, 0, NQ + 7), w_cp(wa_h, 1, 2, NQ + 8), w_cp(wb_h, 0, 2, NQ + 9)]
    woa_cp = cp(woa_h, wo_s.at[pl.ds(0, D)], NQ + 2)
    wob_cp = cp(wob_h, wo_s.at[pl.ds(D, D)], NQ + 3)
    wphi_cp = cp(wphi_h, wphi_s, NQ + 4)
    gate_cp = cp(gate_h, gate_s, NQ + 5)

    wphi_cp.start()
    wbq_cp.start()
    wbk_cp.start()
    xa_cp(0).start()
    xa_cp(1).start()
    late_cp[0].start()
    xa_cp(2).start()
    late_cp[1].start()
    xa_cp(3).start()
    late_cp[2].start()
    wak_cp.start()
    gate_cp.start()
    woa_cp.start()
    wob_cp.start()

    zv[...] = jnp.zeros_like(zv)
    s2[(NQ - 1) % 2] = jnp.zeros((S, TQ), F32)
    (mA, mB)[(NQ - 1) % 2][...] = jnp.zeros((1, TQ), F32)

    wphi_cp.wait()
    for d in range(DH):
        blk = jnp.concatenate(
            [wphi_s[d].astype(F32), jnp.zeros((128 - DH, H), F32)], axis=0)
        f_s[pl.ds(d, H, stride=DH), :] = blk.T
    ranges = ((0, 144), (112, 272), (240, 400), (368, 528), (496, 640))
    fb = f_s[...].astype(BF16)
    bdt = []
    for c, (a, b) in enumerate(ranges):
        rr = jax.lax.broadcasted_iota(I32, (b - a, 128), 0) + a
        ll = jax.lax.broadcasted_iota(I32, (b - a, 128), 1)
        sel = jnp.where(rr % DH == ll, 1.0, 0.0).astype(BF16)
        blk = _dot(sel, fb[128 * c:128 * (c + 1), :], NT)
        bdt.append(jnp.where(rr // DH == (ll + 128 * c) // DH, blk, 0.0).astype(BF16))
    for part in range(2):
        (wbq_cp, wbk_cp)[part].wait()
        acc_s[...] = jnp.zeros_like(acc_s)
        for c, (a, b) in enumerate(ranges):
            wsl = wb_s[:, part * D + 128 * c:part * D + 128 * (c + 1)]
            r = _dot(bdt[c], wsl, NT)
            for n in range(5):
                acc_s[n, a:b, :] += r[:, 128 * n:128 * (n + 1)]
        for j in range(DH):
            for n in range(5):
                r0 = (part * D + H * j) // 2
                wbT[r0:r0 + H // 2, 128 * n:128 * (n + 1)] = _as_u32(
                    (acc_s[n, pl.ds(j, H, stride=DH), :] * LOG2E).astype(BF16))

    def proj_b(c, carry):
        xa_cp(c).wait()

        for k in range(3):
            pl.when(c == k + 1)(late_cp[k].wait)

        sel = jnp.where((c == 1) | (c == 2), 1, 0)
        col0 = jnp.where(c >= 2, 2 * D, 0)
        row0 = jnp.where(c == 3, D + 8, jnp.where(c == 2, D // 2, 0))
        dep = None
        for k in range(5):
            t = _as_u32(w_s[sel, :, pl.ds(pl.multiple_of(col0 + 128 * k, 128), 128)].T)
            wT[pl.ds(pl.multiple_of(row0 + 64 * k, 8), 64), :] = t
            last = t[56:64, :]
            dep = last if dep is None else dep | last
        r0 = pl.multiple_of(c * TQ, TQ)
        x = xa_s[pl.ds(r0, TQ), :]
        vtpA[0:D, pl.ds(r0, TQ)] = _dot(_as_bf16(wbT[0:D // 2, :]), x, NT)
        zrow = jnp.concatenate([pltpu.bitcast(zv[:, 0:128], U32)] * 5, axis=1)
        top = wbT[D // 2:D // 2 + 8, :] | (dep & zrow)
        lhs = jnp.concatenate([top, wbT[D // 2 + 8:D, :]], axis=0)
        vtpA[D:2 * D, pl.ds(r0, TQ)] = _dot(_as_bf16(lhs), x, NT)
        return carry

    jax.lax.fori_loop(0, NQ, proj_b, 0)

    gate_cp.wait()
    wak_cp.wait()
    grow = jax.lax.broadcasted_iota(I32, (16, D), 0)
    wT[D:D + 8, :] = _as_u32(jnp.where(
        grow == 0, jnp.broadcast_to(gate_s[...].astype(F32).reshape(1, D), (16, D)),
        0.0).astype(BF16))

    def feature_maps(c):
        for base, ph_ref in ((0, phq), (D, phk)):
            for t in range(TQ // 128):
                col = pl.ds(pl.multiple_of(c * TQ + t * 128, 128), 128)
                for g in range(H // 8):
                    tile = c * (TQ // 128) + t
                    for sgn in range(2):
                        xs = [vtpA[base + H * j + 8 * g:base + H * j + 8 * (g + 1), col]
                              for j in range(DH)]
                        ext = xs[0]
                        for j in range(1, DH):
                            ext = (jnp.maximum if sgn == 0 else jnp.minimum)(ext, xs[j])
                        es = [jnp.exp2(v - ext if sgn == 0 else ext - v) for v in xs]
                        tot = es[0]
                        for j in range(1, DH):
                            tot = tot + es[j]
                        rr_ = 1.0 / tot
                        for j in range(DH):
                            r = ST * (sgn * DH + j) + 4 * g
                            ph_ref[tile, r:r + 4, :] = pltpu.bitcast((es[j] * rr_).astype(BF16), U32)

    def proj_a(c, carry):
        r0 = pl.multiple_of(c * TQ, TQ)
        x = xa_s[pl.ds(r0, TQ), :]
        k = _dot(x, wa_s[:, D:2 * D])
        kb = k.astype(BF16)
        rh = pl.ds(pl.multiple_of(c * (TQ // 2), TQ // 2), TQ // 2)
        for w in range(5):
            kw[w, rh, :] = _as_u32(kb[:, 128 * w:128 * (w + 1)])
        for w in range(4):
            kw[5 + w, rh, :] = _as_u32(k[:, 64 + 128 * w:192 + 128 * w].astype(BF16))
        feature_maps(c)
        r = _dot(_as_bf16(wT[...]), x, NT)
        qT[:, pl.ds(r0, TQ)] = _as_u32((r[0:D] * QSCALE).astype(BF16))
        vtpA[0:H * 24, pl.ds(r0, TQ)] = _pair_layout(_round_bf16(r[D:2 * D]))
        gl = r[2 * D:2 * D + 8]
        gl = jnp.broadcast_to(gl[0:1], (8, TQ))
        g_s[:, pl.ds(r0, TQ)] = 1.0 / (1.0 + jnp.exp(-gl))
        vtpB[:, pl.ds(r0, TQ)] = _pair_layout(_round_bf16(r[2 * D + 16:3 * D + 16]))
        return carry

    jax.lax.fori_loop(0, NQ, proj_a, 0)

    row24 = jax.lax.broadcasted_iota(I32, (24, TQ), 0)

    def valid24(u):
        return (row24 >= 4 * u) & (row24 < 4 * u + DH)

    def row_start(h, u):
        return pl.multiple_of((h // 2) * 40 + u * 16, 8)

    def load_phi(ph_ref, jp, i):
        n = TQ // 128
        w = jnp.concatenate(
            [ph_ref[i * n + t, pl.ds(jp, 2 * DH, stride=ST), :] for t in range(n)], axis=1)
        return pltpu.bitcast(w, BF16)

    def k_side(jp, i):
        v = vtpB[pl.ds(pl.multiple_of(jp * 48, 8), 48), pl.ds(i * TQ, TQ)]
        return _dot(v, load_phi(phk, jp, i), NT)

    def finish_kv(kv):
        r = jax.lax.broadcasted_iota(I32, kv.shape, 0)
        c = jax.lax.broadcasted_iota(I32, kv.shape, 1)
        return _round_bf16(jnp.where((r >= 24) == (c % 2 == 1), kv, 0.0))

    def special_row(o, u):
        return o[20:21, :] if u == 0 else o[0:1, :]

    def q_side(jp, i, kv):
        res2 = _dot(kv, load_phi(phq, jp, i))
        for u in range(2):
            res = res2[24 * u:24 * (u + 1)]
            o = res * _recip(special_row(res, u) + 1e-6)
            pltpu.store(otB.at[pl.ds(row_start(2 * jp, u), 24), pl.ds(i * TQ, TQ)], o,
                        mask=valid24(u))

    def make_w(h, i):
        c0 = h * DH
        tile = c0 // 128
        rem = c0 - tile * 128
        strad = rem > 128 - DH
        win = jnp.where(strad, 5 + tile, tile)
        off = jnp.where(strad, rem - 64, rem)
        q0 = pl.multiple_of(tile * 64 + jnp.where(strad, 32, 0), 32)
        q32 = qT[pl.ds(q0, 64), pl.ds(i * TQ, TQ)]
        row = jax.lax.broadcasted_iota(I32, (64, TQ), 0) * 2
        msk = (row >= off) & (row < off + DH)
        return win, pltpu.bitcast(jnp.where(msk, q32, jnp.zeros_like(q32)), BF16)

    sbuf = (s2.at[0], s2.at[1])
    mbuf = (mA, mB)

    def run_stages(stages):
        z = zv[...]
        mhist = []
        qst = [dict() for _ in stages]
        pst = [dict() for _ in stages]

        def qk(n, c):
            hq, iq = stages[n][0], stages[n][1]
            st = qst[n]
            if c == 0:
                st["win"], st["w"] = make_w(hq, iq)
            s = _dot(_as_bf16(kw[st["win"], pl.ds(c * CK // 2, CK // 2), :]), st["w"])
            sbuf[iq % 2][pl.ds(c * CK, CK), :] = s
            mx = jnp.max(s.reshape(CK // 8, 8, TQ), axis=0)
            st["m"] = mx if c == 0 else jnp.maximum(st["m"], mx)
            mhist.append(st["m"])
            if c == NC - 1:
                mbuf[iq % 2][...] = jnp.max(st["m"], axis=0, keepdims=True)

        def pv(n, c):
            hp, up, ip, extra = stages[n][2:]
            st = pst[n]
            sl = pl.ds(c * CK, CK)
            if c == 0:
                st["m8"] = jnp.broadcast_to(mbuf[ip % 2][...], (8, TQ))
            me = st["m8"]
            if len(mhist) > SKEW:
                t = pltpu.bitcast(mhist[-1 - SKEW], I32) & z
                me = pltpu.bitcast(pltpu.bitcast(me, I32) | t, F32)
            p = jnp.exp2(sbuf[ip % 2][sl, :].reshape(CK // 8, 8, TQ) - me[None])
            o = _dot(vtpA[pl.ds(pl.multiple_of(hp * 24, 8), 24), sl],
                     p.reshape(CK, TQ).astype(BF16))
            st["o"] = o if c == 0 else st["o"] + o
            if extra is not None and c in extra:
                extra[c]()
            if c == NC - 1:
                o = st["o"] * _recip(special_row(st["o"], up))
                pltpu.store(otA.at[pl.ds(row_start(hp, up), 24), pl.ds(ip * TQ, TQ)], o,
                            mask=valid24(up))

        total = len(stages) * NC
        for pos in range(total + SKEW - 1):
            if pos < total and stages[pos // NC][0] is not None:
                qk(pos // NC, pos % NC)
            back = pos - (SKEW - 1)
            if back >= 0:
                pv(back // NC, back % NC)


    def pair_body(jp, carry):
        kv = [None]
        stages = []
        for u in range(2):
            h = 2 * jp + u
            for i in range(NQ):
                def do_k(i=i):
                    r = k_side(jp, i)
                    kv[0] = r if kv[0] is None else kv[0] + r
                    if i == NQ - 1:
                        kv[0] = finish_kv(kv[0])

                def do_q(i=i):
                    q_side(jp, i, kv[0])

                extra = {MQ: do_k if u == 0 else do_q}
                if i > 0:
                    stages.append((h, i, h, u, i - 1, extra))
                else:
                    stages.append((h, 0, (h + H - 1) % H, 1 - u, NQ - 1, extra))
        run_stages(stages)
        return carry

    jax.lax.fori_loop(0, H // 2, pair_body, 0)

    woa_cp.wait()
    wob_cp.wait()

    def out_cp(r0, size, sem):
        return pltpu.make_async_copy(out_s.at[pl.ds(r0, size)], out_h.at[pl.ds(r0, size)],
                                     osems.at[sem])

    def out_rows(r0, size):
        g = g_s[0:1, pl.ds(r0, size)]
        oa = (otA[:, pl.ds(r0, size)] * g).astype(BF16)
        ob = (otB[:, pl.ds(r0, size)] * (1.0 - g)).astype(BF16)
        o = _dot(jnp.concatenate([oa, ob], axis=0), wo_s[...], TN)
        out_s[pl.ds(r0, size), :] = o.astype(BF16)

    def out_piece(r0, size, sem):
        out_rows(r0, size)
        out_cp(r0, size, sem).start()

    def proj_o(c, carry):
        out_piece(pl.multiple_of(c * TO, TO), TO, c)
        return carry

    run_stages([(None, None, H - 1, 1, NQ - 1, {3: functools.partial(out_rows, 0, TO)})])
    out_cp(0, TO, 0).start()
    n_full = S // TO - 1
    jax.lax.fori_loop(1, n_full, proj_o, 0)
    pieces = [(c * TO, TO) for c in range(n_full)]
    r0 = n_full * TO
    for size in OUT_TAIL:
        out_piece(r0, size, len(pieces))
        pieces.append((r0, size))
        r0 += size
    for n, (r0, size) in enumerate(pieces):
        out_cp(r0, size, n).wait()


@jax.jit
def pallas_gated_mix__mha_block__linear_kernel_hedgehog__prompt_kernel(
    A_x: jax.Array,
    A_wqkv: jax.Array,
    A_wo: jax.Array,
    B_x: jax.Array,
    B_wqkv: jax.Array,
    B_w_phi: jax.Array,
    B_wo: jax.Array,
    gate_w: jax.Array,
):
    xa = A_x.reshape(S, D)
    wphi = B_w_phi.transpose(1, 2, 0)
    any_spec = pl.BlockSpec(memory_space=pl.ANY)
    scratch = [
        pltpu.VMEM((S, D), BF16),
        pltpu.VMEM((2, D, 3 * D), BF16),
        pltpu.VMEM((2 * D, D), BF16),
        pltpu.VMEM((DH, DH, H), BF16),
        pltpu.VMEM((D,), BF16),
        pltpu.VMEM((3 * D // 2 + 8, D), U32),
        pltpu.VMEM((D, D), U32),
        pltpu.VMEM((D, 128), F32),
        pltpu.VMEM((5, D, 128), F32),
        pltpu.VMEM((9, S // 2, 128), U32),
        pltpu.VMEM((D // 2, S), U32),
        pltpu.VMEM((2 * D, S), F32),
        pltpu.VMEM((H * 24, S), F32),
        pltpu.VMEM((8, S), F32),
        pltpu.VMEM((D, S), F32),
        pltpu.VMEM((D, S), F32),
        pltpu.VMEM((2, S, TQ), F32),
        pltpu.VMEM((1, TQ), F32),
        pltpu.VMEM((1, TQ), F32),
        pltpu.VMEM((8, TQ), I32),
        pltpu.VMEM((S // 128, 2 * DH * ST, 128), U32),
        pltpu.VMEM((S // 128, 2 * DH * ST, 128), U32),
        pltpu.VMEM((S, D), BF16),
        pltpu.SemaphoreType.DMA((NQ + 10,)),
        pltpu.SemaphoreType.DMA((S // TO - 1 + len(OUT_TAIL),)),
    ]
    out = pl.pallas_call(
        _kernel,
        out_shape=jax.ShapeDtypeStruct((S, D), BF16),
        in_specs=[any_spec] * 7,
        out_specs=any_spec,
        scratch_shapes=scratch,
        compiler_params=pltpu.CompilerParams(vmem_limit_bytes=110 * 1024 * 1024),
    )(xa, A_wqkv, A_wo, B_wqkv, wphi, B_wo, gate_w)
    return out.reshape(1, S, D)
```
